```python
import os as _os
_os.environ.setdefault('JAX_PLATFORMS', 'cpu')
import jax
import jax.numpy as jnp

def _softmax(x, axis=-1):
    return jax.nn.softmax(x, axis=axis)

def _gelu(x):
    return jax.nn.gelu(x, approximate=True)

def _silu(x):
    return jax.nn.silu(x)

def _sigmoid(x):
    return jax.nn.sigmoid(x)

def _layernorm(x, axis=-1, eps=1e-05):
    m = jnp.mean(x, axis=axis, keepdims=True)
    v = jnp.var(x, axis=axis, keepdims=True)
    return (x - m) / jnp.sqrt(v + eps)

def _scatter_add(tgt, idx, src, axis=0):
    return tgt.at[idx].add(src)

def _segment_sum(src, seg, n):
    return jax.ops.segment_sum(src, seg, n)

class _Rng:

    def __init__(self, key):
        self._k = key

    def _next(self):
        self._k, sub = jax.random.split(self._k)
        return sub

    def normal(self, shape):
        return jax.random.normal(self._next(), shape, dtype=jnp.bfloat16)

    def randint(self, lo, hi, shape):
        return jax.random.randint(self._next(), shape, lo, hi, dtype=jnp.int32)

    def uniform(self, shape, lo=0.0, hi=1.0):
        return jax.random.uniform(self._next(), shape, jnp.bfloat16, lo, hi)

    def permutation(self, n):
        return jax.random.permutation(self._next(), n)
kernel_name = 'adaLN_cond__mha_block_cached__geglu_ffn__prompt'

def setup_inputs():
    _rng = _Rng(jax.random.key(int.from_bytes(__import__("os").urandom(4), "little")))
    _w = lambda a: (lambda t: t.astype(jnp.bfloat16) if jnp.issubdtype(t.dtype, jnp.floating) else t)(jnp.asarray(a))

    def _A_setup():
        B, Sq, D = (1, 2048, 512)
        H, Sk, Dh = (32, 2048, 128)
        return {'x': _w((lambda *s: _rng.normal(s) * 0.05)(B, Sq, D)), 'k_cache': _w((lambda *s: _rng.normal(s) * 3.2)(B, H, Sk, Dh)), 'v_cache': _w((lambda *s: _rng.normal(s) * 0.4)(B, H, Sk, Dh)), 'wq': _w((lambda *s: _rng.normal(s) * 1.6)(D, H * Dh) * D ** (-0.5)), 'wo': _w((lambda *s: _rng.normal(s) * 0.4)(H * Dh, D) * (H * Dh) ** (-0.5))}
    _A_in = _A_setup()

    def _B_setup():
        B, S, D, F = (1, 2048, 512, 1792)
        return {'x': _w((lambda *s: _rng.normal(s) * 0.05)(B, S, D)), 'w_gate': _w((lambda *s: _rng.normal(s) * 0.05)(D, F)), 'w_up': _w((lambda *s: _rng.normal(s) * 0.05)(D, F)), 'w_down': _w((lambda *s: _rng.normal(s) * 0.05)(F, D))}
    _B_in = _B_setup()
    return {'A_x': _A_in['x'], 'A_k_cache': _A_in['k_cache'], 'A_v_cache': _A_in['v_cache'], 'A_wq': _A_in['wq'], 'A_wo': _A_in['wo'], 'B_x': _B_in['x'], 'B_w_gate': _B_in['w_gate'], 'B_w_up': _B_in['w_up'], 'B_w_down': _B_in['w_down'], 'c': _w((lambda *s: _rng.normal(s) * 0.05)(1, 512) * 8.0), 'w_mod': _w((lambda *s: _rng.normal(s) * 0.05)(512, 6 * 512) * 512 ** (-0.5) * 8.0)}

def reference(A_x, A_k_cache, A_v_cache, A_wq, A_wo, B_x, B_w_gate, B_w_up, B_w_down, c, w_mod):

    def _A_ref(x, k_cache, v_cache, wq, wo):
        B, Sq, D = x.shape
        H, Dh = (32, 128)
        q = (lambda x, *d: x.transpose(*d))((x @ wq).reshape(B, Sq, H, Dh), 0, 2, 1, 3)
        scores = jnp.einsum('bhqd,bhkd->bhqk', q, k_cache) * Dh ** (-0.5)
        p = _softmax(scores, axis=-1)
        o = jnp.einsum('bhqk,bhkd->bhqd', p, v_cache)
        return (lambda x, *d: x.transpose(*d))(o, 0, 2, 1, 3).reshape(B, Sq, H * Dh) @ wo

    def _B_ref(x, w_gate, w_up, w_down):
        return _gelu(x @ w_gate) * (x @ w_up) @ w_down
    x = A_x
    mod = (_silu(c) @ w_mod).reshape(c.shape[0], 6, 1, -1)
    sa, ca, ga, sb, cb, gb = (mod[:, 0].copy(), mod[:, 1].copy(), mod[:, 2].copy(), mod[:, 3].copy(), mod[:, 4].copy(), mod[:, 5].copy())
    h = _layernorm(x, axis=-1) * (1 + ca) + sa
    x = x + ga * _A_ref(h, A_k_cache, A_v_cache, A_wq, A_wo)
    h = _layernorm(x, axis=-1) * (1 + cb) + sb
    x = x + gb * _B_ref(h, B_w_gate, B_w_up, B_w_down)
    return x
```

```python
import jax
import jax.numpy as jnp
import jax.experimental.pallas as pl
import jax.experimental.pallas.tpu as pltpu

SEQ = 2048
DM = 512
NH = 32
DH = 128
FF = 1792
TQ = 256
TF = 256
EPS = 1e-05

f32 = jnp.float32
bf16 = jnp.bfloat16


def _ln(x):
    m = jnp.mean(x, axis=-1, keepdims=True)
    xc = x - m
    v = jnp.mean(xc * xc, axis=-1, keepdims=True)
    return xc * jax.lax.rsqrt(v + EPS)


def _gelu_tanh(x):
    c0 = 0.7978845608028654
    return 0.5 * x * (1.0 + jnp.tanh(c0 * (x + 0.044715 * (x * x * x))))


def _kernel(x_ref, k_ref, v_ref, wq_ref, wo_ref, wg_ref, wu_ref, wd_ref,
            c_ref, wmod_ref, o_ref, h_scr, acc_scr, mod_scr, q_scr):
    hd = pl.program_id(0)

    @pl.when(hd == 0)
    def _init():
        c = c_ref[...].astype(f32)
        sc = c * jax.nn.sigmoid(c)
        mod = jnp.dot(sc.astype(bf16), wmod_ref[...], preferred_element_type=f32)
        mod_scr[...] = mod
        sa = mod[:, 0 * DM:1 * DM]
        ca = mod[:, 1 * DM:2 * DM]
        x = x_ref[...].astype(f32)
        h = _ln(x) * (1.0 + ca) + sa
        h_scr[...] = h.astype(bf16)
        acc_scr[...] = jnp.zeros_like(acc_scr)

    scale = DH ** -0.5
    q = jnp.dot(h_scr[...], wq_ref[...], preferred_element_type=f32)
    q_scr[...] = (q * scale).astype(bf16)

    k = k_ref[...]
    v = v_ref[...]
    wo = wo_ref[...]

    def tile(i, carry):
        r0 = pl.multiple_of(i * TQ, TQ)
        qt = q_scr[pl.ds(r0, TQ), :]
        s = jax.lax.dot_general(qt, k, (((1,), (1,)), ((), ())),
                                preferred_element_type=f32)
        m = jnp.max(s, axis=-1, keepdims=True)
        p = jnp.exp(s - m)
        l = jnp.sum(p, axis=-1, keepdims=True)
        o = jnp.dot(p.astype(bf16), v, preferred_element_type=f32)
        o = o * (1.0 / l)
        acc_scr[pl.ds(r0, TQ), :] += jnp.dot(o.astype(bf16), wo,
                                             preferred_element_type=f32)
        return carry

    jax.lax.fori_loop(0, SEQ // TQ, tile, 0)

    @pl.when(hd == NH - 1)
    def _ffn():
        mod = mod_scr[...]
        ga = mod[:, 2 * DM:3 * DM]
        sb = mod[:, 3 * DM:4 * DM]
        cb = mod[:, 4 * DM:5 * DM]
        gb = mod[:, 5 * DM:6 * DM]

        def ftile(i, carry):
            r0 = pl.multiple_of(i * TF, TF)
            x1 = x_ref[pl.ds(r0, TF), :].astype(f32) + ga * acc_scr[pl.ds(r0, TF), :]
            h2 = (_ln(x1) * (1.0 + cb) + sb).astype(bf16)
            g = jnp.dot(h2, wg_ref[...], preferred_element_type=f32)
            u = jnp.dot(h2, wu_ref[...], preferred_element_type=f32)
            a = (_gelu_tanh(g) * u).astype(bf16)
            y = jnp.dot(a, wd_ref[...], preferred_element_type=f32)
            o_ref[pl.ds(r0, TF), :] = (x1 + gb * y).astype(o_ref.dtype)
            return carry

        jax.lax.fori_loop(0, SEQ // TF, ftile, 0)


@jax.jit
def pallas_adaLN_cond__mha_block_cached__geglu_ffn__prompt_kernel(
A_x: jax.Array,
    A_k_cache: jax.Array,
    A_v_cache: jax.Array,
    A_wq: jax.Array,
    A_wo: jax.Array,
    B_x: jax.Array,
    B_w_gate: jax.Array,
    B_w_up: jax.Array,
    B_w_down: jax.Array,
    c: jax.Array,
    w_mod: jax.Array,
):
    x2 = A_x.reshape(SEQ, DM)
    k3 = A_k_cache.reshape(NH, SEQ, DH)
    v3 = A_v_cache.reshape(NH, SEQ, DH)

    const2 = lambda h: (0, 0)
    in_specs = [
        pl.BlockSpec((SEQ, DM), const2),
        pl.BlockSpec((None, SEQ, DH), lambda h: (h, 0, 0)),
        pl.BlockSpec((None, SEQ, DH), lambda h: (h, 0, 0)),
        pl.BlockSpec((DM, DH), lambda h: (0, h)),
        pl.BlockSpec((DH, DM), lambda h: (h, 0)),
        pl.BlockSpec((DM, FF), const2),
        pl.BlockSpec((DM, FF), const2),
        pl.BlockSpec((FF, DM), const2),
        pl.BlockSpec((1, DM), const2),
        pl.BlockSpec((DM, 6 * DM), const2),
    ]
    out = pl.pallas_call(
        _kernel,
        grid=(NH,),
        in_specs=in_specs,
        out_specs=pl.BlockSpec((SEQ, DM), const2),
        out_shape=jax.ShapeDtypeStruct((SEQ, DM), A_x.dtype),
        scratch_shapes=[
            pltpu.VMEM((SEQ, DM), bf16),
            pltpu.VMEM((SEQ, DM), f32),
            pltpu.VMEM((1, 6 * DM), f32),
            pltpu.VMEM((SEQ, DH), bf16),
        ],
        compiler_params=pltpu.CompilerParams(
            dimension_semantics=("arbitrary",),
            vmem_limit_bytes=100 * 1024 * 1024,
        ),
    )(x2, k3, v3, A_wq, A_wo, B_w_gate, B_w_up, B_w_down, c, w_mod)
    return out.reshape(A_x.shape)
```

```python
import jax
import jax.numpy as jnp
import jax.experimental.pallas as pl
import jax.experimental.pallas.tpu as pltpu

SEQ = 2048
DM = 512
NH = 32
DH = 128
FF = 1792

TQ = 512
CB = 512
TF = 256
NXC = 4
XC = SEQ // NXC
NT = SEQ // TQ
NCB = SEQ // CB
NFT = SEQ // TF
EPS = 1e-05

f32 = jnp.float32
bf16 = jnp.bfloat16


def _ln(x):
    m = jnp.mean(x, axis=-1, keepdims=True)
    xc = x - m
    v = jnp.mean(xc * xc, axis=-1, keepdims=True)
    return xc * jax.lax.rsqrt(v + EPS)


def _gelu_tanh(x):
    c0 = 0.7978845608028654
    return 0.5 * x * (1.0 + jnp.tanh(c0 * (x + 0.044715 * (x * x * x))))


def _kernel(x_hbm, k_hbm, v_hbm, wq_hbm, wo_hbm, wg_hbm, wu_hbm, wd_hbm,
            c_ref, wmod_hbm, o_hbm,
            x_ref, k_buf, v_buf, wq_buf, wo_buf, wmod_ref,
            h_scr, acc_scr, q_scr, wg_ref, wu_ref, wd_ref, out_buf,
            xsem, hsem, msem, wsem, osem):
    hd = pl.program_id(0)
    slot = hd % 2

    def late_copies():
        return (pltpu.make_async_copy(wg_hbm, wg_ref, wsem.at[0]),
                pltpu.make_async_copy(wu_hbm, wu_ref, wsem.at[1]),
                pltpu.make_async_copy(wd_hbm, wd_ref, wsem.at[2]),
                pltpu.make_async_copy(wmod_hbm.at[:, 2 * DM:6 * DM],
                                      wmod_ref.at[:, 2 * DM:6 * DM], msem.at[1]))

    def head_copies(h, sl):
        c0 = pl.multiple_of(h * DH, DH)
        return (pltpu.make_async_copy(wq_hbm.at[:, pl.ds(c0, DH)], wq_buf.at[sl],
                                      hsem.at[4 * sl + 0]),
                pltpu.make_async_copy(k_hbm.at[h], k_buf.at[sl], hsem.at[4 * sl + 1]),
                pltpu.make_async_copy(v_hbm.at[h], v_buf.at[sl], hsem.at[4 * sl + 2]),
                pltpu.make_async_copy(wo_hbm.at[pl.ds(c0, DH), :], wo_buf.at[sl],
                                      hsem.at[4 * sl + 3]))

    @pl.when(hd == 0)
    def _init():
        mcp = pltpu.make_async_copy(wmod_hbm.at[:, 0:2 * DM],
                                    wmod_ref.at[:, 0:2 * DM], msem.at[0])
        xcps = [pltpu.make_async_copy(x_hbm.at[t * XC:(t + 1) * XC, :],
                                      x_ref.at[t * XC:(t + 1) * XC, :], xsem.at[t])
                for t in range(NXC)]
        queue = list(xcps[2:]) + list(head_copies(0, 0))
        mcp.start()
        xcps[0].start()
        xcps[1].start()
        acc_scr[...] = jnp.zeros_like(acc_scr)
        c = c_ref[...].astype(f32)
        sc = (c * jax.nn.sigmoid(c)).astype(bf16)
        mcp.wait()
        moda = jnp.dot(sc, wmod_ref[:, 0:2 * DM], preferred_element_type=f32)
        sa = moda[:, 0 * DM:1 * DM]
        ca = moda[:, 1 * DM:2 * DM]
        per = -(-len(queue) // NXC)
        for t in range(NXC):
            xcps[t].wait()
            for cp in queue[t * per:(t + 1) * per]:
                cp.start()
            x = x_ref[t * XC:(t + 1) * XC, :].astype(f32)
            h = _ln(x) * (1.0 + ca) + sa
            h_scr[t * XC:(t + 1) * XC, :] = h.astype(bf16)
        for cp in late_copies():
            cp.start()

    @pl.when(hd + 1 < NH)
    def _prefetch():
        for cp in head_copies(hd + 1, 1 - slot):
            cp.start()

    for cp in head_copies(hd, slot):
        cp.wait()

    q = jnp.dot(h_scr[...], wq_buf[slot], preferred_element_type=f32)
    q_scr[...] = (q * (DH ** -0.5)).astype(bf16)

    k_ref = k_buf.at[slot]
    v_ref = v_buf.at[slot]
    wo = wo_buf[slot]

    m = [None] * NT
    l = [None] * NT
    o = [None] * NT

    def kv_block(i, j):
        r0 = i * TQ
        qt = q_scr[r0:r0 + TQ, :]
        kj = k_ref[j * CB:(j + 1) * CB, :]
        vj = v_ref[j * CB:(j + 1) * CB, :]
        s = jax.lax.dot_general(qt, kj, (((1,), (1,)), ((), ())),
                                preferred_element_type=f32)
        mb = jnp.max(s, axis=-1, keepdims=True)
        if j == 0:
            m[i] = mb
            p = jnp.exp(s - mb)
            l[i] = jnp.sum(p, axis=-1, keepdims=True)
            o[i] = jnp.dot(p.astype(bf16), vj, preferred_element_type=f32)
        else:
            m_new = jnp.maximum(m[i], mb)
            alpha = jnp.exp(m[i] - m_new)
            p = jnp.exp(s - m_new)
            l[i] = alpha * l[i] + jnp.sum(p, axis=-1, keepdims=True)
            o[i] = alpha * o[i] + jnp.dot(p.astype(bf16), vj,
                                          preferred_element_type=f32)
            m[i] = m_new

    def finish_tile(i):
        r0 = i * TQ
        oo = o[i] * (1.0 / l[i])
        acc_scr[r0:r0 + TQ, :] += jnp.dot(oo.astype(bf16), wo,
                                          preferred_element_type=f32)

    for i in range(NT):
        for j in range(NCB):
            kv_block(i, j)
            if i > 0 and j == 0:
                finish_tile(i - 1)
    finish_tile(NT - 1)

    @pl.when(hd == NH - 1)
    def _ffn():
        for cp in late_copies():
            cp.wait()
        c = c_ref[...].astype(f32)
        sc = (c * jax.nn.sigmoid(c)).astype(bf16)
        modb = jnp.dot(sc, wmod_ref[:, 2 * DM:6 * DM], preferred_element_type=f32)
        ga = modb[:, 0 * DM:1 * DM]
        sb = modb[:, 1 * DM:2 * DM]
        cb = modb[:, 2 * DM:3 * DM]
        gb = modb[:, 3 * DM:4 * DM]

        def out_copy(i):
            r0 = pl.multiple_of(i * TF, TF)
            return pltpu.make_async_copy(out_buf.at[pl.ds(r0, TF), :],
                                         o_hbm.at[pl.ds(r0, TF), :], osem.at[i])

        def ftile(i, carry):
            r0 = pl.multiple_of(i * TF, TF)
            x1 = x_ref[pl.ds(r0, TF), :].astype(f32) + ga * acc_scr[pl.ds(r0, TF), :]
            h2 = (_ln(x1) * (1.0 + cb) + sb).astype(bf16)
            g = jnp.dot(h2, wg_ref[...], preferred_element_type=f32)
            u = jnp.dot(h2, wu_ref[...], preferred_element_type=f32)
            a = (_gelu_tanh(g) * u).astype(bf16)
            y = jnp.dot(a, wd_ref[...], preferred_element_type=f32)
            out_buf[pl.ds(r0, TF), :] = (x1 + gb * y).astype(out_buf.dtype)
            out_copy(i).start()
            return carry

        jax.lax.fori_loop(0, NFT, ftile, 0, unroll=4)
        for i in range(NFT):
            out_copy(i).wait()


@jax.jit
def pallas_adaLN_cond__mha_block_cached__geglu_ffn__prompt_kernel(
A_x: jax.Array,
    A_k_cache: jax.Array,
    A_v_cache: jax.Array,
    A_wq: jax.Array,
    A_wo: jax.Array,
    B_x: jax.Array,
    B_w_gate: jax.Array,
    B_w_up: jax.Array,
    B_w_down: jax.Array,
    c: jax.Array,
    w_mod: jax.Array,
):
    x2 = A_x.reshape(SEQ, DM)
    k3 = A_k_cache.reshape(NH, SEQ, DH)
    v3 = A_v_cache.reshape(NH, SEQ, DH)

    hbm = pl.BlockSpec(memory_space=pl.ANY)
    in_specs = [hbm, hbm, hbm, hbm, hbm, hbm, hbm, hbm,
                pl.BlockSpec((1, DM), lambda h: (0, 0)),
                hbm]
    out = pl.pallas_call(
        _kernel,
        grid=(NH,),
        in_specs=in_specs,
        out_specs=hbm,
        out_shape=jax.ShapeDtypeStruct((SEQ, DM), A_x.dtype),
        scratch_shapes=[
            pltpu.VMEM((SEQ, DM), bf16),
            pltpu.VMEM((2, SEQ, DH), bf16),
            pltpu.VMEM((2, SEQ, DH), bf16),
            pltpu.VMEM((2, DM, DH), bf16),
            pltpu.VMEM((2, DH, DM), bf16),
            pltpu.VMEM((DM, 6 * DM), bf16),
            pltpu.VMEM((SEQ, DM), bf16),
            pltpu.VMEM((SEQ, DM), f32),
            pltpu.VMEM((SEQ, DH), bf16),
            pltpu.VMEM((DM, FF), bf16),
            pltpu.VMEM((DM, FF), bf16),
            pltpu.VMEM((FF, DM), bf16),
            pltpu.VMEM((SEQ, DM), bf16),
            pltpu.SemaphoreType.DMA((NXC,)),
            pltpu.SemaphoreType.DMA((8,)),
            pltpu.SemaphoreType.DMA((2,)),
            pltpu.SemaphoreType.DMA((3,)),
            pltpu.SemaphoreType.DMA((NFT,)),
        ],
        compiler_params=pltpu.CompilerParams(
            dimension_semantics=("arbitrary",),
            vmem_limit_bytes=100 * 1024 * 1024,
        ),
    )(x2, k3, v3, A_wq, A_wo, B_w_gate, B_w_up, B_w_down, c, w_mod)
    return out.reshape(A_x.shape)
```
